```python
import os as _os
_os.environ.setdefault("JAX_PLATFORMS", "cpu")
import jax
import jax.numpy as jnp

def _softmax(x, axis=-1):
    return jax.nn.softmax(x, axis=axis)
def _gelu(x):
    return jax.nn.gelu(x, approximate=True)
def _silu(x):
    return jax.nn.silu(x)
def _sigmoid(x):
    return jax.nn.sigmoid(x)
def _layernorm(x, axis=-1, eps=1e-5):
    m = jnp.mean(x, axis=axis, keepdims=True)
    v = jnp.var(x, axis=axis, keepdims=True)
    return (x - m) / jnp.sqrt(v + eps)
def _scatter_add(tgt, idx, src, axis=0):
    return tgt.at[idx].add(src)
def _segment_sum(src, seg, n):
    return jax.ops.segment_sum(src, seg, n)
class _Rng:
    def __init__(self, key):
        self._k = key
    def _next(self):
        self._k, sub = jax.random.split(self._k)
        return sub
    def normal(self, shape):
        return jax.random.normal(self._next(), shape, dtype=jnp.bfloat16)
    def randint(self, lo, hi, shape):
        return jax.random.randint(self._next(), shape, lo, hi, dtype=jnp.int32)
    def uniform(self, shape, lo=0.0, hi=1.0):
        return jax.random.uniform(self._next(), shape, jnp.bfloat16, lo, hi)
    def permutation(self, n):
        return jax.random.permutation(self._next(), n)


kernel_name = 'gated_mix__linear_kernel_hedgehog__mixer_s_mlp__prompt'

def setup_inputs():
    _rng = _Rng(jax.random.key(int.from_bytes(__import__("os").urandom(4), "little")))
    _w = (lambda a: (lambda t: t.astype(jnp.bfloat16) if jnp.issubdtype(t.dtype, jnp.floating) else t)(jnp.asarray(a)))
    def _A_setup():
        B, S, D, H = 1, 2048, 512, 32
        Dh = D // H
        return {
            "x": _w((lambda *s: _rng.normal(s) * 0.05)(B, S, D)),
            "wqkv": _w((lambda *s: _rng.normal(s) * 1.6)(D, 3 * D)),
            "w_phi": _w((lambda *s: _rng.normal(s) * 1.6)(H, Dh, Dh) * (Dh ** -0.5)),
            "wo": _w((lambda *s: _rng.normal(s) * 0.05)(D, D)),
        }
    _A_in = _A_setup()

    def _B_setup():
        B, S, D, F = 1, 2048, 512, 1376
        return {
            "x":  _w((lambda *s: _rng.normal(s) * 0.05)(B, S, D)),
            "w1": _w((lambda *s: _rng.normal(s) * 0.4)(D, D) * (D ** -0.5)),
            "w2": _w((lambda *s: _rng.normal(s) * 0.4)(D, D) * (D ** -0.5)),
            "w3": _w((lambda *s: _rng.normal(s) * 0.4)(D, F) * (D ** -0.5)),
            "w4": _w((lambda *s: _rng.normal(s) * 0.4)(F, D) * (F ** -0.5)),
        }
    _B_in = _B_setup()

    return {
        "A_x": _A_in["x"],
        "A_wqkv": _A_in["wqkv"],
        "A_w_phi": _A_in["w_phi"],
        "A_wo": _A_in["wo"],
        "B_x": _B_in["x"],
        "B_w1": _B_in["w1"],
        "B_w2": _B_in["w2"],
        "B_w3": _B_in["w3"],
        "B_w4": _B_in["w4"],
        "gate_w": _w((lambda *s: _rng.normal(s) * 0.05)(512) * 16.0),
    }

def reference(A_x, A_wqkv, A_w_phi, A_wo, B_x, B_w1, B_w2, B_w3, B_w4, gate_w):
    def _A_ref(x, wqkv, w_phi, wo):
        B, S, D = x.shape
        H = 32; Dh = D // H
        qkv = (lambda x, *d: x.transpose(*d))((x @ wqkv).reshape(B, S, 3, H, Dh), 2, 0, 3, 1, 4)
        q, k, v = qkv[0], qkv[1], qkv[2]
        pq = jnp.einsum("bhsd,hdf->bhsf", q, w_phi)
        pk = jnp.einsum("bhsd,hdf->bhsf", k, w_phi)
        phi_q = jnp.concatenate([_softmax(pq, axis=-1), _softmax(-pq, axis=-1)], axis=-1)
        phi_k = jnp.concatenate([_softmax(pk, axis=-1), _softmax(-pk, axis=-1)], axis=-1)
        kv = jnp.einsum("bhsf,bhsd->bhfd", phi_k, v)
        z  = jnp.einsum("bhsf->bhf", phi_k)
        num = jnp.einsum("bhqf,bhfd->bhqd", phi_q, kv)
        den = jnp.einsum("bhqf,bhf->bhq", phi_q, z)[..., None] + 1e-6
        o = num / den
        return (lambda x, *d: x.transpose(*d))(o, 0, 2, 1, 3).reshape(B, S, D) @ wo

    def _B_ref(x, w1, w2, w3, w4):
        B, S, D = x.shape
        h = _gelu(_layernorm(x, axis=-1) @ w1)
        c = D // 4
        g0 = jnp.pad(h[:, :, 0*c:1*c], ((0, 0), (1, 0), (0, 0)))[:, :S, :]
        g1 = jnp.pad(h[:, :, 1*c:2*c], ((0, 0), (0, 1), (0, 0)))[:, 1:, :]
        g2 = jnp.pad(h[:, :, 2*c:3*c], ((0, 0), (2, 0), (0, 0)))[:, :S, :]
        g3 = jnp.pad(h[:, :, 3*c:   ], ((0, 0), (0, 2), (0, 0)))[:, 2:, :]
        hs = jnp.concatenate([g0, g1, g2, g3], axis=-1) @ w2
        x1 = x + hs
        h2 = _gelu(_layernorm(x1, axis=-1) @ w3) @ w4
        return x1 + h2

    x = A_x
    g = _sigmoid((x * gate_w).sum(-1, keepdims=True))
    a = _A_ref(x, A_wqkv, A_w_phi, A_wo)
    b = _B_ref(x, B_w1, B_w2, B_w3, B_w4)
    return g * a + (1 - g) * b
```

```python
import functools
import jax
import jax.numpy as jnp
from jax import lax
import jax.experimental.pallas as pl
import jax.experimental.pallas.tpu as pltpu

S, D, H, DH, F = 2048, 512, 32, 16, 1376
NC = D // 128
T = 256
NT = S // T
PAD = 8
LOG2E = 1.4426950408889634
GC1 = 0.7978845608028654
GC2 = GC1 * 0.044715
NT_DIMS = (((1,), (1,)), ((), ()))
f32, bf16 = jnp.float32, jnp.bfloat16


def _gelu(u):
    return 0.5 * u * (1.0 + jnp.tanh(u * (GC1 + GC2 * (u * u))))


def _ln(u):
    m = jnp.mean(u, axis=-1, keepdims=True)
    c = u - m
    v = jnp.mean(c * c, axis=-1, keepdims=True)
    return c * lax.rsqrt(v + 1e-5)


def _dual_exp(p):
    p3 = p.reshape(DH, 8, p.shape[-1])
    mx = jnp.max(p3, axis=0)
    mn = jnp.min(p3, axis=0)
    ep = jnp.exp2(p3 - mx[None])
    en = jnp.exp2(mn[None] - p3)
    return ep, en, jnp.sum(ep, axis=0), jnp.sum(en, axis=0)


def _kernel(x_hbm, wqkv_hbm, wphi_hbm, wo_hbm, w1_hbm, w2_hbm, w3_hbm, w4_hbm, gate_hbm,
            out_hbm,
            x_s, wq_s, wk_s, wv_s, wphi_s, wo_s, w1_s, w2_s, w3_s, w4_s, gate_s,
            wqT_s, wkT_s, h_s, kv_s, z_s, kvT_s, out_s,
            xsem, wsem, osem):
    def xcp(t):
        return pltpu.make_async_copy(x_hbm.at[0, pl.ds(t * T, T), :], x_s.at[pl.ds(t * T, T), :], xsem.at[t])

    def ocp(t):
        return pltpu.make_async_copy(out_s.at[pl.ds(t * T, T), :], out_hbm.at[0, pl.ds(t * T, T), :], osem.at[t])

    cps = dict(
        wphi=pltpu.make_async_copy(wphi_hbm, wphi_s, wsem.at[0]),
        wk=pltpu.make_async_copy(wqkv_hbm.at[:, pl.ds(D, D)], wk_s, wsem.at[1]),
        wv=pltpu.make_async_copy(wqkv_hbm.at[:, pl.ds(2 * D, D)], wv_s, wsem.at[2]),
        w1=pltpu.make_async_copy(w1_hbm, w1_s, wsem.at[3]),
        wq=pltpu.make_async_copy(wqkv_hbm.at[:, pl.ds(0, D)], wq_s, wsem.at[4]),
        w2=pltpu.make_async_copy(w2_hbm, w2_s, wsem.at[5]),
        w3=pltpu.make_async_copy(w3_hbm, w3_s, wsem.at[6]),
        w4=pltpu.make_async_copy(w4_hbm, w4_s, wsem.at[7]),
        wo=pltpu.make_async_copy(wo_hbm, wo_s, wsem.at[8]),
        gate=pltpu.make_async_copy(gate_hbm, gate_s, wsem.at[9]),
    )
    cps['wphi'].start()
    cps['wk'].start()
    xcp(0).start()
    cps['wv'].start()
    cps['w1'].start()
    for t in range(1, NT):
        xcp(t).start()
    for n in ('wq', 'gate', 'w2', 'w3', 'w4', 'wo'):
        cps[n].start()

    h_s[:, pl.ds(0, PAD), :] = jnp.zeros((NC, PAD, 128), f32)
    h_s[:, pl.ds(PAD + S, PAD), :] = jnp.zeros((NC, PAD, 128), f32)
    kv_s[...] = jnp.zeros(kv_s.shape, f32)
    z_s[...] = jnp.zeros(z_s.shape, f32)

    row = lax.broadcasted_iota(jnp.int32, (128, 128), 0)
    col = lax.broadcasted_iota(jnp.int32, (128, 128), 1)
    head_mask = (row % 8) == (col // DH)
    sel = jnp.where(lax.broadcasted_iota(jnp.int32, (H, D), 0) == lax.broadcasted_iota(jnp.int32, (H, D), 1) // DH,
                    1.0, 0.0).astype(bf16)
    dmask = (lax.broadcasted_iota(jnp.int32, (256, D), 0) // DH) == (lax.broadcasted_iota(jnp.int32, (256, D), 1) % DH)
    e2 = jnp.where(lax.broadcasted_iota(jnp.int32, (128, 256), 0) // 8 == lax.broadcasted_iota(jnp.int32, (128, 256), 1) % DH,
                   1.0, 0.0).astype(bf16)

    cps['wphi'].wait()
    a2d = wphi_s[...].reshape(DH * DH, H)
    bm = jnp.where(dmask, jnp.dot(a2d, sel, preferred_element_type=f32), 0.0).astype(bf16)
    pall = jnp.dot(e2, bm, preferred_element_type=f32)
    pts = [jnp.where(head_mask, pall[:, c * 128:(c + 1) * 128], 0.0).astype(bf16) for c in range(NC)]

    def fold(w_s, wT_s):
        for c in range(NC):
            r = lax.dot_general(pts[c], w_s[:, c * 128:(c + 1) * 128], NT_DIMS, preferred_element_type=f32)
            wT_s[c * 128:(c + 1) * 128, :] = (r * LOG2E).astype(bf16)

    cps['wk'].wait()
    fold(wk_s, wkT_s)
    cps['wv'].wait()
    cps['w1'].wait()

    def phase1(t, carry):
        xcp(t).wait()
        r0 = pl.multiple_of(t * T, T)
        xt = x_s[pl.ds(r0, T), :]
        pkT = lax.dot_general(wkT_s[...], xt, NT_DIMS, preferred_element_type=f32)
        v = jnp.dot(xt, wv_s[...], preferred_element_type=f32).astype(bf16)
        for c in range(NC):
            ep, en, sp, sn = _dual_exp(pkT[c * 128:(c + 1) * 128])
            php = ep * (1.0 / sp)[None]
            phn = en * (1.0 / sn)[None]
            ph = jnp.concatenate([php.reshape(128, T), phn.reshape(128, T)], axis=0)
            z_s[c] += ph
            kv_s[c] += jnp.dot(ph.astype(bf16), v[:, c * 128:(c + 1) * 128], preferred_element_type=f32)
        hh = _gelu(jnp.dot(_ln(xt.astype(f32)).astype(bf16), w1_s[...], preferred_element_type=f32))
        for c in range(NC):
            h_s[c, pl.ds(r0 + PAD, T), :] = hh[:, c * 128:(c + 1) * 128]
        return carry

    lax.fori_loop(0, NT, phase1, 0)

    cps['wq'].wait()
    fold(wq_s, wqT_s)
    mask2 = jnp.concatenate([head_mask, head_mask], axis=0)
    for c in range(NC):
        kvT_s[c] = jnp.where(mask2, kv_s[c], 0.0).T.astype(bf16)
        z_s[c] = jnp.broadcast_to(jnp.sum(z_s[c], axis=1, keepdims=True), (256, T))
    for n in ('gate', 'w2', 'w3', 'w4', 'wo'):
        cps[n].wait()

    shifts = (-1, 1, -2, 2)

    def phase2(t, carry):
        r0 = pl.multiple_of(t * T, T)
        xt = x_s[pl.ds(r0, T), :]
        xf = xt.astype(f32)
        pqT = lax.dot_general(wqT_s[...], xt, NT_DIMS, preferred_element_type=f32)
        oTs = []
        for c in range(NC):
            ep, en, sp, sn = _dual_exp(pqT[c * 128:(c + 1) * 128])
            z = z_s[c]
            zp = z[:128].reshape(DH, 8, T)
            zn = z[128:].reshape(DH, 8, T)
            rp = 1.0 / sp
            rn = 1.0 / sn
            den = jnp.sum(ep * zp, axis=0) * rp + jnp.sum(en * zn, axis=0) * rn + 1e-6
            rd = 1.0 / den
            php = ep * (rp * rd)[None]
            phn = en * (rn * rd)[None]
            ph = jnp.concatenate([php.reshape(128, T), phn.reshape(128, T)], axis=0).astype(bf16)
            oTs.append(jnp.dot(kvT_s[c], ph, preferred_element_type=f32))
        o = jnp.concatenate(oTs, axis=0).T.astype(bf16)
        a = jnp.dot(o, wo_s[...], preferred_element_type=f32)
        hsh = jnp.concatenate(
            [h_s[c, pl.ds(r0 + PAD + shifts[c], T), :].astype(bf16) for c in range(NC)], axis=1)
        x1 = xf + jnp.dot(hsh, w2_s[...], preferred_element_type=f32)
        u = _gelu(lax.dot_general(_ln(x1).astype(bf16), w3_s[...], NT_DIMS, preferred_element_type=f32))
        b = x1 + jnp.dot(u.astype(bf16), w4_s[...], preferred_element_type=f32)
        g = jax.nn.sigmoid(jnp.sum(xf * gate_s[...].astype(f32).reshape(1, D), axis=-1, keepdims=True))
        out_s[pl.ds(r0, T), :] = (b + g * (a - b)).astype(bf16)
        ocp(t).start()
        return carry

    lax.fori_loop(0, NT, phase2, 0)
    for t in range(NT):
        ocp(t).wait()


@jax.jit
def pallas_gated_mix__linear_kernel_hedgehog__mixer_s_mlp__prompt_kernel(
    A_x, A_wqkv, A_w_phi, A_wo, B_x, B_w1, B_w2, B_w3, B_w4, gate_w,
):
    any_spec = pl.BlockSpec(memory_space=pltpu.HBM)
    return pl.pallas_call(
        _kernel,
        out_shape=jax.ShapeDtypeStruct((1, S, D), bf16),
        in_specs=[any_spec] * 9,
        out_specs=any_spec,
        scratch_shapes=[
            pltpu.VMEM((S, D), bf16),
            pltpu.VMEM((D, D), bf16), pltpu.VMEM((D, D), bf16), pltpu.VMEM((D, D), bf16),
            pltpu.VMEM((DH, DH, H), bf16),
            pltpu.VMEM((D, D), bf16), pltpu.VMEM((D, D), bf16), pltpu.VMEM((D, D), bf16),
            pltpu.VMEM((F, D), bf16), pltpu.VMEM((F, D), bf16),
            pltpu.VMEM((D,), bf16),
            pltpu.VMEM((D, D), bf16), pltpu.VMEM((D, D), bf16),
            pltpu.VMEM((NC, S + 2 * PAD, 128), f32),
            pltpu.VMEM((NC, 256, 128), f32),
            pltpu.VMEM((NC, 256, T), f32),
            pltpu.VMEM((NC, 128, 256), bf16),
            pltpu.VMEM((S, D), bf16),
            pltpu.SemaphoreType.DMA((NT,)),
            pltpu.SemaphoreType.DMA((10,)),
            pltpu.SemaphoreType.DMA((NT,)),
        ],
        compiler_params=pltpu.CompilerParams(vmem_limit_bytes=64 * 1024 * 1024),
    )(A_x, A_wqkv, jnp.transpose(A_w_phi, (1, 2, 0)), A_wo, B_w1, B_w2, B_w3.T, B_w4, gate_w)
```

```python
import os
import jax
import jax.numpy as jnp
from jax import lax
import jax.experimental.pallas as pl
import jax.experimental.pallas.tpu as pltpu

S, D, H, DH, F = 2048, 512, 32, 16, 1376
NC = D // 128
NG = 8
T0 = 512
T1 = int(os.environ.get('KT1', 256))
T = int(os.environ.get('KT', 256))
W1SPLIT = int(os.environ.get('KW1S', 2))
OSPLIT = int(os.environ.get('KOS', 4))
GPH = int(os.environ.get('KGPH', 2))
LN1P = int(os.environ.get('KLN1P', 1))
NT = S // T
ORDER = os.environ.get('KORD', 'w2.0,w2.1,w3.0,w4a.0,pq.0,w4b.0,oT.0,w3.1,wo.0,pq.1,w4a.1,oT.1,w4b.1,wo.1')
ORD1 = os.environ.get('KORD1', 'pv.0,w1.0,kv.0,pv.1,w1.1,kv.1,pv.2,w1.2,kv.2,pv.3,w1.3,kv.3,pv.4,w1.4,kv.4,fq.0,pv.5,kv.5,w1.5')
ORD0 = os.environ.get('KORD0', 'pk.0,vt.0,pv.1,kv.0,kv.1')
PAD = 8
LOG2E = 1.4426950408889634
GC1 = 0.7978845608028654
GC2 = GC1 * 0.044715
NT_DIMS = (((1,), (1,)), ((), ()))
f32, bf16, u32 = jnp.float32, jnp.bfloat16, jnp.uint32
PR = 480


def _pk(v):
    return pltpu.bitcast(v, u32)


def _upk(v):
    return pltpu.bitcast(v, bf16)


def _gelu(u, half=0.5):
    return (u * half) * (1.0 + jnp.tanh(u * (GC1 + GC2 * (u * u))))


RSQ = int(os.environ.get('KRSQ', 1))
RCP = int(os.environ.get('KRCP', 0))


def _gelu_h(v):
    return v + v * jnp.tanh(v * (2.0 * GC1 + (8.0 * GC2) * (v * v)))


def _recip(x):
    if RCP == 1:
        r = pl.reciprocal(x, approx=True)
        return r * (2.0 - x * r)
    if RCP == 2:
        return jnp.exp2(-jnp.log2(x))
    return 1.0 / x


def _ln(u, half=False):
    m = jnp.sum(u, axis=-1, keepdims=True) * (1.0 / D)
    if LN1P:
        v = jnp.maximum(jnp.sum(u * u, axis=-1, keepdims=True) * (1.0 / D) - m * m, 0.0) + 1e-5
        if RSQ:
            l = jnp.log2(v) * -0.5
            r = jnp.exp2(l - 1.0 if half else l)
        else:
            r = lax.rsqrt(v * 4.0 if half else v)
        return (u - m) * r
    c = u - m
    v = jnp.sum(c * c, axis=-1, keepdims=True) * (1.0 / D)
    return c * lax.rsqrt(v + 1e-5)


def _fsum(e):
    s = jnp.sum(e, axis=0)
    return s + pltpu.roll(s, 4, 0)


def _group(p, j):
    n = p.shape[-1]
    c, g2 = j // 2, j % 2
    main = p[c * 120 + g2 * 64:c * 120 + g2 * 64 + 56].reshape(7, 8, n)
    sub = lax.broadcasted_iota(jnp.int32, (8, n), 0)
    keep = (sub < 4) if g2 == 0 else (sub >= 4)
    last = jnp.where(keep, p[c * 120 + 56:c * 120 + 64], 0.0)
    return jnp.concatenate([main, last[None]], axis=0)


def _dual_exp(p3):
    mx = jnp.max(p3, axis=0)
    mx = jnp.maximum(mx, pltpu.roll(mx, 4, 0))
    mn = jnp.min(p3, axis=0)
    mn = jnp.minimum(mn, pltpu.roll(mn, 4, 0))
    ep = jnp.exp2(p3 - mx[None])
    en = jnp.exp2(mn[None] - p3)
    return ep, en, _fsum(ep), _fsum(en)


def _iota(shape, dim):
    return lax.broadcasted_iota(jnp.int32, shape, dim)


def _kernel(x_hbm, wqkv_hbm, wphi_hbm, wo_hbm, w1_hbm, w2_hbm, w3_hbm, w4_hbm, gate_hbm,
            out_hbm,
            x_s, wq_s, wk_s, wv_s, wphi_s, wo_s, w1_s, w2_s, w3_s, w4_s, gate_s,
            wqT_s, wkvT_s, h_s, kv_s, z_s, kvT_s, out_s, pt_s,
            wsem):
    TO = T // OSPLIT

    def ocp(r, n):
        return pltpu.make_async_copy(out_s.at[pl.ds(r, n), :], out_hbm.at[0, pl.ds(r, n), :], wsem.at[0])

    W1C = D // W1SPLIT
    cps = dict(
        wphi=pltpu.make_async_copy(wphi_hbm, wphi_s, wsem.at[0]),
        wk=pltpu.make_async_copy(wqkv_hbm.at[:, pl.ds(D, D)], wk_s, wsem.at[4]),
        wv=pltpu.make_async_copy(wqkv_hbm.at[:, pl.ds(2 * D, D)], wv_s, wsem.at[4]),
        wq=pltpu.make_async_copy(wqkv_hbm.at[:, pl.ds(0, D)], wq_s, wsem.at[5]),
        w2=pltpu.make_async_copy(w2_hbm, w2_s, wsem.at[6]),
        w3=pltpu.make_async_copy(w3_hbm, w3_s, wsem.at[6]),
        w4=pltpu.make_async_copy(w4_hbm, w4_s, wsem.at[6]),
        wo=pltpu.make_async_copy(wo_hbm, wo_s, wsem.at[6]),
        gate=pltpu.make_async_copy(gate_hbm, gate_s, wsem.at[6]),
        xb=pltpu.make_async_copy(x_hbm.at[0, pl.ds(T0, S - T0), :], x_s.at[pl.ds(T0, S - T0), :], wsem.at[5]),
    )
    w1cp = [pltpu.make_async_copy(w1_hbm.at[:, pl.ds(i * W1C, W1C)], w1_s.at[:, pl.ds(i * W1C, W1C)], wsem.at[2 + i])
            for i in range(W1SPLIT)]
    XSPLIT = 2
    XA = T0 // XSPLIT
    xacp = [pltpu.make_async_copy(x_hbm.at[0, pl.ds(i * XA, XA), :], x_s.at[pl.ds(i * XA, XA), :], wsem.at[i])
            for i in range(XSPLIT)]
    cps['wphi'].start()
    for c in xacp:
        c.start()
    for c in w1cp:
        c.start()
    for n in ('wk', 'wv', 'xb', 'wq', 'w2', 'w3', 'w4', 'wo', 'gate'):
        cps[n].start()

    h_s[:, pl.ds(0, PAD), :] = jnp.zeros((NC, PAD, 128), f32)
    h_s[:, pl.ds(PAD + S, PAD), :] = jnp.zeros((NC, PAD, 128), f32)

    def ln_x(r0, n):
        return _ln(x_s[pl.ds(r0, n), :].astype(f32), True).astype(bf16)

    def h_part(ln, r0, n, c0, c1):
        hh = _gelu_h(jnp.dot(ln, w1_s[:, c0 * 128:c1 * 128], preferred_element_type=f32))
        for c in range(c0, c1):
            h_s[c, pl.ds(r0 + PAD, n), :] = hh[:, (c - c0) * 128:(c - c0 + 1) * 128]

    def fold(w_s, wT_s):
        lo = _iota((8, D), 0) < 4
        rows = []
        for c in range(NC):
            r = lax.dot_general(pt_s[c], w_s[:, c * 128:(c + 1) * 128], NT_DIMS, preferred_element_type=f32) * LOG2E
            a7, b7 = r[56:64], r[120:128]
            a7r, b7r = pltpu.roll(a7, 4, 0), pltpu.roll(b7, 4, 0)
            ra = jnp.where(lo, a7r, a7)
            rb = jnp.where(lo, b7, b7r)
            rows.append((r[0:56].reshape(7, 8, D) - ra[None]).reshape(56, D))
            rows.append(jnp.where(lo, a7 - a7r, b7 - b7r))
            rows.append((r[64:120].reshape(7, 8, D) - rb[None]).reshape(56, D))
        wT_s[0:PR // 2, :] = _pk(jnp.concatenate(rows, axis=0).astype(bf16))

    def s_pk(c):
        c['pk'] = lax.dot_general(_upk(wkvT_s[0:PR // 2, :]), x_s[pl.ds(c['r0'], c['n']), :], NT_DIMS,
                                  preferred_element_type=f32)

    def s_vt(c):
        c['vt'] = lax.dot_general(_upk(wkvT_s[PR // 2:(PR + D) // 2, :]), x_s[pl.ds(c['r0'], c['n']), :], NT_DIMS,
                                  preferred_element_type=f32)

    def s_pv(c):
        pv = lax.dot_general(_upk(wkvT_s[...]), x_s[pl.ds(c['r0'], c['n']), :], NT_DIMS, preferred_element_type=f32)
        c['pk'] = pv[:PR]
        c['vt'] = pv[PR:]

    def s_w1(c):
        h_part(ln_x(c['r0'], c['n']), c['r0'], c['n'], 0, NC)

    def s_kv(c):
        n = c['n']
        for j in range(NG):
            ep, en, sp, sn = _dual_exp(_group(c['pk'], j))
            r = _recip(sp * sn)
            php = ep * (r * sn)[None]
            phn = en * (r * sp)[None]
            ph = jnp.concatenate([php.reshape(64, n), phn.reshape(64, n)], axis=0)
            zz = ph[:, 0:128]
            for i in range(1, n // 128):
                zz = zz + ph[:, i * 128:(i + 1) * 128]
            kk = lax.dot_general(c['vt'][j * 64:(j + 1) * 64].astype(bf16), ph.astype(bf16), NT_DIMS, preferred_element_type=f32)
            if c['first']:
                z_s[j] = zz
                kv_s[j] = kk
            else:
                z_s[j] += zz
                kv_s[j] += kk

    st1 = dict(pk=s_pk, vt=s_vt, pv=s_pv, w1=s_w1, kv=s_kv, fq=lambda c: fold(wq_s, wqT_s))

    row = _iota((128, 128), 0)
    head_mask = ((row >> 6) * 4 + (row & 3)) == (_iota((128, 128), 1) >> 4)
    sel = jnp.where(_iota((H, D), 0) == (_iota((H, D), 1) >> 4), 1.0, 0.0).astype(bf16)
    dmask = (_iota((256, D), 0) >> 4) == (_iota((256, D), 1) & 15)
    e2 = jnp.where(((_iota((128, 256), 0) & 63) >> 2) == (_iota((128, 256), 1) & 15), 1.0, 0.0).astype(bf16)
    cps['wphi'].wait()
    xacp[0].wait()
    a2d = wphi_s[...].reshape(DH * DH, H)
    bm = jnp.where(dmask, jnp.dot(a2d, sel, preferred_element_type=f32), 0.0).astype(bf16)
    lns = [ln_x(0, XA)]
    for i in range(1, XSPLIT):
        xacp[i].wait()
        if i == 1:
            pall = jnp.dot(e2, bm, preferred_element_type=f32)
            for c in range(NC):
                pt_s[c] = jnp.where(head_mask, pall[:, c * 128:(c + 1) * 128], 0.0).astype(bf16)
        lns.append(ln_x(i * XA, XA))
    ln0 = jnp.concatenate(lns, axis=0)
    cw = NC // W1SPLIT
    for i in range(W1SPLIT):
        w1cp[i].wait()
        h_part(ln0, 0, T0, i * cw, (i + 1) * cw)

    cps['wk'].wait()
    cps['wv'].wait()
    fold(wk_s, wkvT_s)
    wkvT_s[PR // 2:(PR + D) // 2, :] = _pk(wv_s[...].T)
    o0 = [o.split('.') for o in ORD0.split(',')]
    n0 = max(int(o[1]) for o in o0) + 1
    c0 = [dict(r0=k * (T0 // n0), n=T0 // n0, first=(k == 0)) for k in range(n0)]
    for name, k in o0:
        st1[name](c0[int(k)])
    cps['xb'].wait()
    cps['wq'].wait()

    n1 = (S - T0) // T1
    c1 = [dict(r0=T0 + k * T1, n=T1, first=False) for k in range(n1)]
    if '.' in ORD1:
        o1 = [o.split('.') for o in ORD1.split(',')]
    else:
        o1 = []
        pat = ORD1.split(',')
        for k in range(n1 + 1):
            for p in pat:
                nm, lag = (p[:-2], 1) if p.endswith('-1') else (p, 0)
                if 0 <= k - lag < n1:
                    o1.append((nm, k - lag))
        pos = int(os.environ.get('KFQ', 0))
        o1.insert(len(o1) - pos, ('fq', 0))
    for name, k in o1:
        st1[name](c1[int(k)])

    kmask = (_iota((64, 128), 0) >> 4) == (_iota((64, 128), 1) & 3)
    for j in range(NG):
        kvT_s[j] = _pk(jnp.where(kmask, kv_s[j], 0.0).astype(bf16))
        z_s[j] = jnp.broadcast_to(jnp.sum(z_s[j], axis=1, keepdims=True), (128, 128))
    for n in ('w2', 'w3', 'w4', 'wo', 'gate'):
        cps[n].wait()

    shifts = (-1, 1, -2, 2)

    def gate_parts(c):
        hw = gate_s[...].astype(f32).reshape(1, D) * 0.5
        th = jnp.tanh(jnp.sum(c['xt'].astype(f32) * hw, axis=-1, keepdims=True))
        c['gg'] = 0.5 + 0.5 * th
        c['ng'] = 0.5 - 0.5 * th

    def st_w2(c):
        r0 = c['r0']
        hsh = jnp.concatenate(
            [h_s[k, pl.ds(r0 + PAD + shifts[k], T), :] for k in range(NC)], axis=1).astype(bf16)
        c['x1'] = c['xt'].astype(f32) + jnp.dot(hsh, w2_s[...], preferred_element_type=f32)
        c['ln'] = _ln(c['x1'], GPH != 3).astype(bf16)
        gate_parts(c)

    def st_w3(c, lo, hi):
        u = lax.dot_general(c['ln'], w3_s[lo:hi, :], NT_DIMS, preferred_element_type=f32)
        c.setdefault('u', {})[lo] = (_gelu(u, 0.5 * c['ng']) if GPH == 3 else _gelu_h(u)).astype(bf16)

    def st_pq(c):
        c['pqT'] = lax.dot_general(_upk(wqT_s[...]), c['xt'], NT_DIMS, preferred_element_type=f32)

    def st_oT(c):
        oTs = []
        for j in range(NG):
            ep, en, sp, sn = _dual_exp(_group(c['pqT'], j))
            z = jnp.concatenate([z_s[j]] * (T // 128), axis=1)
            zp = z[:64].reshape(8, 8, T)
            zn = z[64:].reshape(8, 8, T)
            dd = _fsum(ep * zp) * sn + (_fsum(en * zn) + 1e-6 * sn) * sp
            rd = _recip(dd)
            php = ep * (sn * rd)[None]
            phn = en * (sp * rd)[None]
            ph = jnp.concatenate([php.reshape(64, T), phn.reshape(64, T)], axis=0).astype(bf16)
            oTs.append(jnp.dot(_upk(kvT_s[j]), ph, preferred_element_type=f32))
        c['o'] = jnp.concatenate(oTs, axis=0).T.astype(bf16)

    def st_w4(c, nlo, nhi, klo=0, khi=F):
        us = [v for k, v in sorted(c['u'].items()) if klo <= k < khi]
        u = us[0] if len(us) == 1 else jnp.concatenate(us, axis=1)
        assert u.shape[1] == khi - klo
        r = jnp.dot(u, w4_s[klo:khi, nlo:nhi], preferred_element_type=f32)
        b = c.setdefault('b', {})
        if nlo in b:
            b[nlo] = b[nlo] + r
        else:
            b[nlo] = (c['x1'][:, nlo:nhi] * c['ng'] if GPH == 3 else c['x1'][:, nlo:nhi]) + r

    def st_wo(c):
        bs = [v for k, v in sorted(c['b'].items())]
        b = bs[0] if len(bs) == 1 else jnp.concatenate(bs, axis=1)
        r0 = c['r0']
        osp = OSPLIT if c['last'] else 1
        to = T // osp
        for i in range(osp):
            a = jnp.dot(c['o'][i * to:(i + 1) * to], wo_s[...], preferred_element_type=f32)
            bi = b[i * to:(i + 1) * to]
            g = c['gg'][i * to:(i + 1) * to]
            res = bi + g * a if GPH == 3 else bi + g * (a - bi)
            out_s[pl.ds(r0 + i * to, to), :] = res.astype(bf16)
            ocp(r0 + i * to, to).start()

    FH = 768
    stages = {
        'w2': st_w2, 'pq': st_pq, 'oT': st_oT, 'wo': st_wo,
        'w3': lambda c: st_w3(c, 0, F), 'w3a': lambda c: st_w3(c, 0, FH), 'w3b': lambda c: st_w3(c, FH, F),
        'w4': lambda c: st_w4(c, 0, 512),
        'w4a': lambda c: st_w4(c, 0, 256), 'w4b': lambda c: st_w4(c, 256, 512),
        'w4p': lambda c: st_w4(c, 0, 128), 'w4q': lambda c: st_w4(c, 128, 256),
        'w4r': lambda c: st_w4(c, 256, 384), 'w4s': lambda c: st_w4(c, 384, 512),
        'w4x': lambda c: st_w4(c, 0, 512, 0, FH), 'w4y': lambda c: st_w4(c, 0, 512, FH, F),
    }
    order = [o.split('.') for o in ORDER.split(',')]
    ntile = max(int(o[1]) for o in order) + 1

    def phase2(i, carry):
        cs = []
        for k in range(ntile):
            r0 = pl.multiple_of((i * ntile + k) * T, T)
            cs.append(dict(r0=r0, xt=x_s[pl.ds(r0, T), :], last=(k == ntile - 1)))
        for name, k in order:
            stages[name](cs[int(k)])
        return carry

    lax.fori_loop(0, NT // ntile, phase2, 0)
    pltpu.make_async_copy(out_s, out_hbm.at[0], wsem.at[0]).wait()


@jax.jit
def pallas_gated_mix__linear_kernel_hedgehog__mixer_s_mlp__prompt_kernel(
    A_x, A_wqkv, A_w_phi, A_wo, B_x, B_w1, B_w2, B_w3, B_w4, gate_w,
):
    any_spec = pl.BlockSpec(memory_space=pltpu.HBM)
    return pl.pallas_call(
        _kernel,
        out_shape=jax.ShapeDtypeStruct((1, S, D), bf16),
        in_specs=[any_spec] * 9,
        out_specs=any_spec,
        scratch_shapes=[
            pltpu.VMEM((S, D), bf16),
            pltpu.VMEM((D, D), bf16), pltpu.VMEM((D, D), bf16), pltpu.VMEM((D, D), bf16),
            pltpu.VMEM((DH, DH, H), bf16),
            pltpu.VMEM((D, D), bf16), pltpu.VMEM((D, D), bf16), pltpu.VMEM((D, D), bf16),
            pltpu.VMEM((F, D), bf16), pltpu.VMEM((F, D), bf16),
            pltpu.VMEM((D,), bf16),
            pltpu.VMEM((PR // 2, D), u32), pltpu.VMEM(((PR + D) // 2, D), u32),
            pltpu.VMEM((NC, S + 2 * PAD, 128), f32),
            pltpu.VMEM((NG, 64, 128), f32),
            pltpu.VMEM((NG, 128, 128), f32),
            pltpu.VMEM((NG, 32, 128), u32),
            pltpu.VMEM((S, D), bf16),
            pltpu.VMEM((NC, 128, 128), bf16),
            pltpu.SemaphoreType.DMA((7,)),
        ],
        compiler_params=pltpu.CompilerParams(vmem_limit_bytes=64 * 1024 * 1024, disable_bounds_checks=True,
                                             disable_semaphore_checks=True),
    )(A_x, A_wqkv, jnp.transpose(A_w_phi, (1, 2, 0)), A_wo, B_w1, B_w2, B_w3.T, B_w4, gate_w)
```

```python
import jax
import jax.numpy as jnp
from jax import lax
import jax.experimental.pallas as pl
import jax.experimental.pallas.tpu as pltpu

S, D, H, DH, F = 2048, 512, 32, 16, 1376
NC = D // 128
NG = 8
T = 256
NT = S // T
OSPLIT = 4
PAD = 8
PR = 480
FM = 1280
HD = D // 2
LOG2E = 1.4426950408889634
GC1 = 0.7978845608028654
GC2 = GC1 * 0.044715
NT_DIMS = (((1,), (1,)), ((), ()))
f32, bf16, u32 = jnp.float32, jnp.bfloat16, jnp.uint32

PHASE1 = (
    'W:wphi,P1,W:x0-1,P2,ln.0,W:w1a,w1a.0,W:wka,fa,pka.0,sma.0,W:wkb+w1b,fb,pkb.0,w1b.0,smb.0,'
    'W:x1-2+wv,wvT,pk.1,vt.0,kv.0,w1a.1,vt.1,kv.1,W:x2-8+wq,w1b.1,'
    'pv.2,w1.2,kv.2,pv.3,w1.3,kv.3,pv.4,w1.4,kv.4,pv.5,w1.5,kv.5,pv.6,w1.6,kv.6,fq,pv.7,kv.7,w1.7,'
    'FIN,W:w2+w3+w4+wo+gate').split(',')
PHASE2 = (
    'w2.0,w2.1,w3m.0,w3t.0,w4a.0,pq.0,w4b.0,oT.0,w2.2,w3t.1,wo.0,w3m.1,w4a.1,pq.1,w4b.1,oT.1,'
    'w2.3,w3m.2,wo.1,w3t.2,w4a.2,pq.2,w4b.2,oT.2,w3t.3,w3m.3,pq.3,wo.2,w4a.3,oT.3,w4b.3,wo.3').split(',')
TILES_PER_STEP = 4
NSEM = sum(t.startswith('W:') for t in PHASE1)


def _pk(v):
    return pltpu.bitcast(v, u32)


def _upk(v):
    return pltpu.bitcast(v, bf16)


def _iota(shape, dim):
    return lax.broadcasted_iota(jnp.int32, shape, dim)


def _gelu_h(v):
    return v + v * jnp.tanh(v * (2.0 * GC1 + (8.0 * GC2) * (v * v)))


def _ln_h(u):
    m = jnp.sum(u, axis=-1, keepdims=True) * (1.0 / D)
    v = jnp.maximum(jnp.sum(u * u, axis=-1, keepdims=True) * (1.0 / D) - m * m, 0.0) + 1e-5
    return (u - m) * jnp.exp2(jnp.log2(v) * -0.5 - 1.0)


def _fsum(e):
    s = jnp.sum(e, axis=0)
    return s + pltpu.roll(s, 4, 0)


def _group(p, j):
    n = p.shape[-1]
    c, g2 = j // 2, j % 2
    main = p[c * 120 + g2 * 64:c * 120 + g2 * 64 + 56].reshape(7, 8, n)
    sub = _iota((8, n), 0)
    keep = (sub < 4) if g2 == 0 else (sub >= 4)
    last = jnp.where(keep, p[c * 120 + 56:c * 120 + 64], 0.0)
    return jnp.concatenate([main, last[None]], axis=0)


def _dual_exp(p3):
    mx = jnp.max(p3, axis=0)
    mx = jnp.maximum(mx, pltpu.roll(mx, 4, 0))
    mn = jnp.min(p3, axis=0)
    mn = jnp.minimum(mn, pltpu.roll(mn, 4, 0))
    ep = jnp.exp2(p3 - mx[None])
    en = jnp.exp2(mn[None] - p3)
    return ep, en, _fsum(ep), _fsum(en)


def _kernel(x_hbm, wqkv_hbm, wphi_hbm, wo_hbm, w1_hbm, w2_hbm, w3_hbm, w4_hbm, gate_hbm,
            out_hbm,
            x_s, wq_s, wk_s, wv_s, wphi_s, wo_s, w1_s, w2_s, w3_s, w4_s, gate_s,
            wqT_s, wkvT_s, h_s, kv_s, z_s, kvT_s, out_s, pt_s,
            sems):
    def in_copy(name, sem):
        if name[0] == 'x':
            a, b = (int(v) for v in name[1:].split('-'))
            rows = pl.ds(a * T, (b - a) * T)
            return pltpu.make_async_copy(x_hbm.at[0, rows, :], x_s.at[rows, :], sem)
        src, dst = dict(
            wphi=(wphi_hbm, wphi_s),
            wka=(wqkv_hbm.at[:, pl.ds(D, HD)], wk_s.at[:, pl.ds(0, HD)]),
            wkb=(wqkv_hbm.at[:, pl.ds(D + HD, HD)], wk_s.at[:, pl.ds(HD, HD)]),
            wv=(wqkv_hbm.at[:, pl.ds(2 * D, D)], wv_s),
            wq=(wqkv_hbm.at[:, pl.ds(0, D)], wq_s),
            w1a=(w1_hbm.at[:, pl.ds(0, HD)], w1_s.at[:, pl.ds(0, HD)]),
            w1b=(w1_hbm.at[:, pl.ds(HD, HD)], w1_s.at[:, pl.ds(HD, HD)]),
            w2=(w2_hbm, w2_s), w3=(w3_hbm, w3_s), w4=(w4_hbm, w4_s), wo=(wo_hbm, wo_s),
            gate=(gate_hbm, gate_s),
        )[name]
        return pltpu.make_async_copy(src, dst, sem)

    waits = [t for t in PHASE1 if t.startswith('W:')]
    groups = [[in_copy(n, sems.at[i]) for n in t[2:].split('+')] for i, t in enumerate(waits)]
    for grp in groups:
        for cp in grp:
            cp.start()

    h_s[:, pl.ds(0, PAD), :] = jnp.zeros((NC, PAD, 128), f32)
    h_s[:, pl.ds(PAD + S, PAD), :] = jnp.zeros((NC, PAD, 128), f32)

    tmp = {}

    def s_p1():
        sel = jnp.where(_iota((H, D), 0) == (_iota((H, D), 1) >> 4), 1.0, 0.0).astype(bf16)
        dmask = (_iota((256, D), 0) >> 4) == (_iota((256, D), 1) & 15)
        a2d = wphi_s[...].reshape(DH * DH, H)
        tmp['bm'] = jnp.where(dmask, jnp.dot(a2d, sel, preferred_element_type=f32), 0.0).astype(bf16)

    def s_p2():
        row = _iota((128, 128), 0)
        head_mask = ((row >> 6) * 4 + (row & 3)) == (_iota((128, 128), 1) >> 4)
        e2 = jnp.where(((_iota((128, 256), 0) & 63) >> 2) == (_iota((128, 256), 1) & 15), 1.0, 0.0).astype(bf16)
        pall = jnp.dot(e2, tmp['bm'], preferred_element_type=f32)
        for c in range(NC):
            pt_s[c] = jnp.where(head_mask, pall[:, c * 128:(c + 1) * 128], 0.0).astype(bf16)

    def fold(w_s, wT_s, c0, c1):
        lo = _iota((8, D), 0) < 4
        rows = []
        for c in range(c0, c1):
            r = lax.dot_general(pt_s[c], w_s[:, c * 128:(c + 1) * 128], NT_DIMS,
                                preferred_element_type=f32) * LOG2E
            a7, b7 = r[56:64], r[120:128]
            a7r, b7r = pltpu.roll(a7, 4, 0), pltpu.roll(b7, 4, 0)
            ra = jnp.where(lo, a7r, a7)
            rb = jnp.where(lo, b7, b7r)
            rows.append((r[0:56].reshape(7, 8, D) - ra[None]).reshape(56, D))
            rows.append(jnp.where(lo, a7 - a7r, b7 - b7r))
            rows.append((r[64:120].reshape(7, 8, D) - rb[None]).reshape(56, D))
        wT_s[c0 * 60:c1 * 60, :] = _pk(jnp.concatenate(rows, axis=0).astype(bf16))

    def s_wvT():
        wkvT_s[PR // 2:(PR + D) // 2, :] = _pk(wv_s[...].T)

    def xt(c):
        return x_s[pl.ds(c['r0'], T), :]

    def proj(lo, hi, c):
        return lax.dot_general(_upk(wkvT_s[lo // 2:hi // 2, :]), xt(c), NT_DIMS, preferred_element_type=f32)

    def s_pk(c):
        p = proj(0, PR, c)
        c['pka'], c['pkb'] = p[:PR // 2], p[PR // 2:]

    def s_pka(c):
        c['pka'] = proj(0, PR // 2, c)

    def s_pkb(c):
        c['pkb'] = proj(PR // 2, PR, c)

    def s_vt(c):
        c['vt'] = proj(PR, PR + D, c)

    def s_pv(c):
        p = proj(0, PR + D, c)
        c['pka'], c['pkb'], c['vt'] = p[:PR // 2], p[PR // 2:PR], p[PR:]

    def s_ln(c):
        c['ln'] = _ln_h(xt(c).astype(f32)).astype(bf16)

    def s_w1(c, c0=0, c1=NC):
        if 'ln' not in c:
            s_ln(c)
        hh = _gelu_h(jnp.dot(c['ln'], w1_s[:, c0 * 128:c1 * 128], preferred_element_type=f32))
        for k in range(c0, c1):
            h_s[k, pl.ds(c['r0'] + PAD, T), :] = hh[:, (k - c0) * 128:(k - c0 + 1) * 128]

    z_seen, kv_seen = set(), set()

    def sm_group(c, j):
        ep, en, sp, sn = _dual_exp(_group(c['pka'] if j < 4 else c['pkb'], j % 4))
        r = 1.0 / (sp * sn)
        php = ep * (r * sn)[None]
        phn = en * (r * sp)[None]
        ph = jnp.concatenate([php.reshape(64, T), phn.reshape(64, T)], axis=0)
        zz = ph[:, 0:128] + ph[:, 128:256]
        if j in z_seen:
            z_s[j] += zz
        else:
            z_s[j] = zz
            z_seen.add(j)
        c.setdefault('ph', {})[j] = ph.astype(bf16)

    def s_kv(c):
        for j in range(NG):
            if j not in c.get('ph', {}):
                sm_group(c, j)
            kk = lax.dot_general(c['vt'][j * 64:(j + 1) * 64].astype(bf16), c['ph'][j], NT_DIMS,
                                 preferred_element_type=f32)
            if j in kv_seen:
                kv_s[j] += kk
            else:
                kv_s[j] = kk
                kv_seen.add(j)

    def s_fin():
        kmask = (_iota((64, 128), 0) >> 4) == (_iota((64, 128), 1) & 3)
        for j in range(NG):
            kvT_s[j] = _pk(jnp.where(kmask, kv_s[j], 0.0).astype(bf16))
            z_s[j] = jnp.broadcast_to(jnp.sum(z_s[j], axis=1, keepdims=True), (128, 128))

    global_stage = dict(
        P1=s_p1, P2=s_p2, wvT=s_wvT, FIN=s_fin,
        fa=lambda: fold(wk_s, wkvT_s, 0, 2), fb=lambda: fold(wk_s, wkvT_s, 2, 4),
        fq=lambda: fold(wq_s, wqT_s, 0, 4))
    tile_stage = dict(
        pk=s_pk, pka=s_pka, pkb=s_pkb, vt=s_vt, pv=s_pv, ln=s_ln, w1=s_w1, kv=s_kv,
        w1a=lambda c: s_w1(c, 0, 2), w1b=lambda c: s_w1(c, 2, 4),
        sma=lambda c: [sm_group(c, j) for j in range(4)],
        smb=lambda c: [sm_group(c, j) for j in range(4, 8)])
    tiles = [dict(r0=k * T) for k in range(NT)]
    pending = iter(groups)
    for tok in PHASE1:
        if tok.startswith('W:'):
            for cp in next(pending):
                cp.wait()
        elif '.' in tok:
            name, k = tok.split('.')
            tile_stage[name](tiles[int(k)])
        else:
            global_stage[tok]()

    shifts = (-1, 1, -2, 2)

    def st_w2(c):
        r0 = c['r0']
        hsh = jnp.concatenate(
            [h_s[k, pl.ds(r0 + PAD + shifts[k], T), :] for k in range(NC)], axis=1).astype(bf16)
        c['x1'] = c['xt'].astype(f32) + jnp.dot(hsh, w2_s[...], preferred_element_type=f32)
        c['ln'] = _ln_h(c['x1']).astype(bf16)

    def st_w3m(c):
        u = lax.dot_general(c['ln'], w3_s[0:FM, :], NT_DIMS, preferred_element_type=f32)
        c['um'] = _gelu_h(u).astype(bf16)

    def st_w3t(c):
        ut = lax.dot_general(w3_s[FM:F, :], c['ln'], NT_DIMS, preferred_element_type=f32)
        ut = jnp.concatenate([_gelu_h(ut), jnp.zeros((128 - (F - FM), T), f32)], axis=0)
        c['ut'] = ut.T[:, :F - FM].astype(bf16)

    def st_pq(c):
        c['pqT'] = lax.dot_general(_upk(wqT_s[...]), c['xt'], NT_DIMS, preferred_element_type=f32)

    def st_oT(c):
        oTs = []
        for j in range(NG):
            ep, en, sp, sn = _dual_exp(_group(c['pqT'], j))
            z = jnp.concatenate([z_s[j]] * (T // 128), axis=1)
            zp = z[:64].reshape(8, 8, T)
            zn = z[64:].reshape(8, 8, T)
            dd = _fsum(ep * zp) * sn + (_fsum(en * zn) + 1e-6 * sn) * sp
            rd = 1.0 / dd
            php = ep * (sn * rd)[None]
            phn = en * (sp * rd)[None]
            ph = jnp.concatenate([php.reshape(64, T), phn.reshape(64, T)], axis=0).astype(bf16)
            oTs.append(jnp.dot(_upk(kvT_s[j]), ph, preferred_element_type=f32))
        hw = gate_s[...].astype(f32).reshape(1, D) * 0.5
        th = jnp.tanh(jnp.sum(c['xt'].astype(f32) * hw, axis=-1, keepdims=True))
        c['ng'] = 0.5 - 0.5 * th
        c['o'] = (jnp.concatenate(oTs, axis=0).T * (0.5 + 0.5 * th)).astype(bf16)

    def st_w4(c, key, nlo, nhi):
        u = jnp.concatenate([c['um'], c['ut']], axis=1)
        c[key] = c['x1'][:, nlo:nhi] + jnp.dot(u, w4_s[:, nlo:nhi], preferred_element_type=f32)

    def st_wo(c):
        b = jnp.concatenate([c['ba'], c['bb']], axis=1)
        pieces = OSPLIT if c['last'] else 1
        n = T // pieces
        for i in range(pieces):
            a = jnp.dot(c['o'][i * n:(i + 1) * n], wo_s[...], preferred_element_type=f32)
            rows = pl.ds(c['r0'] + i * n, n)
            out_s[rows, :] = (b[i * n:(i + 1) * n] * c['ng'][i * n:(i + 1) * n] + a).astype(bf16)
            pltpu.make_async_copy(out_s.at[rows, :], out_hbm.at[0, rows, :], sems.at[0]).start()

    stage2 = dict(w2=st_w2, w3m=st_w3m, w3t=st_w3t, pq=st_pq, oT=st_oT, wo=st_wo,
                  w4a=lambda c: st_w4(c, 'ba', 0, HD), w4b=lambda c: st_w4(c, 'bb', HD, D))

    def phase2(i, carry):
        cs = []
        for k in range(TILES_PER_STEP):
            r0 = pl.multiple_of((i * TILES_PER_STEP + k) * T, T)
            cs.append(dict(r0=r0, xt=x_s[pl.ds(r0, T), :], last=(k == TILES_PER_STEP - 1)))
        for tok in PHASE2:
            name, k = tok.split('.')
            stage2[name](cs[int(k)])
        return carry

    lax.fori_loop(0, NT // TILES_PER_STEP, phase2, 0)
    pltpu.make_async_copy(out_s, out_hbm.at[0], sems.at[0]).wait()


@jax.jit
def pallas_gated_mix__linear_kernel_hedgehog__mixer_s_mlp__prompt_kernel(
    A_x: jax.Array,
    A_wqkv: jax.Array,
    A_w_phi: jax.Array,
    A_wo: jax.Array,
    B_x: jax.Array,
    B_w1: jax.Array,
    B_w2: jax.Array,
    B_w3: jax.Array,
    B_w4: jax.Array,
    gate_w: jax.Array,
):
    del B_x
    hbm = pl.BlockSpec(memory_space=pltpu.HBM)
    return pl.pallas_call(
        _kernel,
        out_shape=jax.ShapeDtypeStruct((1, S, D), bf16),
        in_specs=[hbm] * 9,
        out_specs=hbm,
        scratch_shapes=[
            pltpu.VMEM((S, D), bf16),
            pltpu.VMEM((D, D), bf16), pltpu.VMEM((D, D), bf16), pltpu.VMEM((D, D), bf16),
            pltpu.VMEM((DH, DH, H), bf16),
            pltpu.VMEM((D, D), bf16), pltpu.VMEM((D, D), bf16), pltpu.VMEM((D, D), bf16),
            pltpu.VMEM((F, D), bf16), pltpu.VMEM((F, D), bf16),
            pltpu.VMEM((D,), bf16),
            pltpu.VMEM((PR // 2, D), u32), pltpu.VMEM(((PR + D) // 2, D), u32),
            pltpu.VMEM((NC, S + 2 * PAD, 128), f32),
            pltpu.VMEM((NG, 64, 128), f32),
            pltpu.VMEM((NG, 128, 128), f32),
            pltpu.VMEM((NG, 32, 128), u32),
            pltpu.VMEM((S, D), bf16),
            pltpu.VMEM((NC, 128, 128), bf16),
            pltpu.SemaphoreType.DMA((NSEM,)),
        ],
        compiler_params=pltpu.CompilerParams(
            vmem_limit_bytes=64 * 1024 * 1024,
            disable_bounds_checks=True,
            disable_semaphore_checks=True,
        ),
    )(A_x, A_wqkv, jnp.transpose(A_w_phi, (1, 2, 0)), A_wo, B_w1, B_w2, B_w3.T, B_w4, gate_w)
```

```python
import jax
import jax.numpy as jnp
from jax import lax
import jax.experimental.pallas as pl
import jax.experimental.pallas.tpu as pltpu

S, D, H, DH, F = 2048, 512, 32, 16, 1376
NC = D // 128
NG = 8
T = 256
NT = S // T
CUTS = (0, 128, 192, 224, 256)
PAD = 8
PR = 480
FM = 1280
HD = D // 2
LOG2E = 1.4426950408889634
GC1 = 0.7978845608028654
GC2 = GC1 * 0.044715
NT_DIMS = (((1,), (1,)), ((), ()))
f32, bf16, u32 = jnp.float32, jnp.bfloat16, jnp.uint32

PHASE1 = (
    'W:wphi,P1,W:x0-1,P2,ln.0,W:w1a,w1a.0,W:wka,fa,pka.0,sma.0,W:wkb+w1b,fb,pkb.0,w1b.0,smb.0,'
    'W:x1-2+wv,wvT,pk.1,vt.0,w1a.1,vt.1,kv.0,kv.1,W:x2-8+wq,w1b.1,'
    'pv.2,w1a.2,w1b.2,pv.3,w1.3,kv.2,w1.4,kv.3,pv.4,w1.5,kv.4,pv.5,w1.6,kv.5,pv.6,w1.7,kv.6,pv.7,fq,kv.7,'
    'FIN,W:w2+w3+w4+wo+gate').split(',')
PHASE2 = (
    'w2.0,w2.1,w3m.0,w3t.0,w4a.0,pq.0,w4b.0,oT.0,w2.2,w3t.1,wo.0,w3m.1,w4a.1,pq.1,w4b.1,oT.1,'
    'w2.3,w3m.2,wo.1,w3t.2,w4a.2,pq.2,w4b.2,oT.2,w3t.3,w3m.3,pq.3,wo.2,w4a.3,oT.3,w4b.3,wo.3').split(',')
TILES_PER_STEP = 4
NSEM = sum(t.startswith('W:') for t in PHASE1)


def _pk(v):
    return pltpu.bitcast(v, u32)


def _upk(v):
    return pltpu.bitcast(v, bf16)


def _iota(shape, dim):
    return lax.broadcasted_iota(jnp.int32, shape, dim)


def _gelu_h(v):
    return v + v * jnp.tanh(v * (2.0 * GC1 + (8.0 * GC2) * (v * v)))


def _ln_h(u):
    m = jnp.sum(u, axis=-1, keepdims=True) * (1.0 / D)
    v = jnp.maximum(jnp.sum(u * u, axis=-1, keepdims=True) * (1.0 / D) - m * m, 0.0) + 1e-5
    return (u - m) * jnp.exp2(jnp.log2(v) * -0.5 - 1.0)


def _fsum(e):
    s = jnp.sum(e, axis=0)
    return s + pltpu.roll(s, 4, 0)


def _group(p, j):
    n = p.shape[-1]
    c, g2 = j // 2, j % 2
    main = p[c * 120 + g2 * 64:c * 120 + g2 * 64 + 56].reshape(7, 8, n)
    sub = _iota((8, n), 0)
    keep = (sub < 4) if g2 == 0 else (sub >= 4)
    last = jnp.where(keep, p[c * 120 + 56:c * 120 + 64], 0.0)
    return jnp.concatenate([main, last[None]], axis=0)


def _dual_exp(p3):
    mx = jnp.max(p3, axis=0)
    mx = jnp.maximum(mx, pltpu.roll(mx, 4, 0))
    mn = jnp.min(p3, axis=0)
    mn = jnp.minimum(mn, pltpu.roll(mn, 4, 0))
    ep = jnp.exp2(p3 - mx[None])
    en = jnp.exp2(mn[None] - p3)
    return ep, en, _fsum(ep), _fsum(en)


def _kernel(x_hbm, wqkv_hbm, wphi_hbm, wo_hbm, w1_hbm, w2_hbm, w3_hbm, w4_hbm, gate_hbm,
            out_hbm,
            x_s, wq_s, wk_s, wv_s, wphi_s, wo_s, w1_s, w2_s, w3_s, w4_s, gate_s,
            wqT_s, wkvT_s, h_s, kv_s, z_s, kvT_s, out_s, pt_s,
            sems):
    def in_copy(name, sem):
        if name[0] == 'x':
            a, b = (int(v) for v in name[1:].split('-'))
            rows = pl.ds(a * T, (b - a) * T)
            return pltpu.make_async_copy(x_hbm.at[0, rows, :], x_s.at[rows, :], sem)
        src, dst = dict(
            wphi=(wphi_hbm, wphi_s),
            wka=(wqkv_hbm.at[:, pl.ds(D, HD)], wk_s.at[:, pl.ds(0, HD)]),
            wkb=(wqkv_hbm.at[:, pl.ds(D + HD, HD)], wk_s.at[:, pl.ds(HD, HD)]),
            wv=(wqkv_hbm.at[:, pl.ds(2 * D, D)], wv_s),
            wq=(wqkv_hbm.at[:, pl.ds(0, D)], wq_s),
            w1a=(w1_hbm.at[:, pl.ds(0, HD)], w1_s.at[:, pl.ds(0, HD)]),
            w1b=(w1_hbm.at[:, pl.ds(HD, HD)], w1_s.at[:, pl.ds(HD, HD)]),
            w2=(w2_hbm, w2_s), w3=(w3_hbm, w3_s), w4=(w4_hbm, w4_s), wo=(wo_hbm, wo_s),
            gate=(gate_hbm, gate_s),
        )[name]
        return pltpu.make_async_copy(src, dst, sem)

    waits = [t for t in PHASE1 if t.startswith('W:')]
    groups = [[in_copy(n, sems.at[i]) for n in t[2:].split('+')] for i, t in enumerate(waits)]
    for grp in groups:
        for cp in grp:
            cp.start()

    h_s[:, pl.ds(0, PAD), :] = jnp.zeros((NC, PAD, 128), f32)
    h_s[:, pl.ds(PAD + S, PAD), :] = jnp.zeros((NC, PAD, 128), f32)

    tmp = {}

    def s_p1():
        sel = jnp.where(_iota((H, D), 0) == (_iota((H, D), 1) >> 4), 1.0, 0.0).astype(bf16)
        dmask = (_iota((256, D), 0) >> 4) == (_iota((256, D), 1) & 15)
        a2d = wphi_s[...].reshape(DH * DH, H)
        tmp['bm'] = jnp.where(dmask, jnp.dot(a2d, sel, preferred_element_type=f32), 0.0).astype(bf16)

    def s_p2():
        row = _iota((128, 128), 0)
        head_mask = ((row >> 6) * 4 + (row & 3)) == (_iota((128, 128), 1) >> 4)
        e2 = jnp.where(((_iota((128, 256), 0) & 63) >> 2) == (_iota((128, 256), 1) & 15), 1.0, 0.0).astype(bf16)
        pall = jnp.dot(e2, tmp['bm'], preferred_element_type=f32)
        for c in range(NC):
            pt_s[c] = jnp.where(head_mask, pall[:, c * 128:(c + 1) * 128], 0.0).astype(bf16)

    def fold(w_s, wT_s, c0, c1):
        lo = _iota((8, D), 0) < 4
        rows = []
        for c in range(c0, c1):
            r = lax.dot_general(pt_s[c], w_s[:, c * 128:(c + 1) * 128], NT_DIMS,
                                preferred_element_type=f32) * LOG2E
            a7, b7 = r[56:64], r[120:128]
            a7r, b7r = pltpu.roll(a7, 4, 0), pltpu.roll(b7, 4, 0)
            ra = jnp.where(lo, a7r, a7)
            rb = jnp.where(lo, b7, b7r)
            rows.append((r[0:56].reshape(7, 8, D) - ra[None]).reshape(56, D))
            rows.append(jnp.where(lo, a7 - a7r, b7 - b7r))
            rows.append((r[64:120].reshape(7, 8, D) - rb[None]).reshape(56, D))
        wT_s[c0 * 60:c1 * 60, :] = _pk(jnp.concatenate(rows, axis=0).astype(bf16))

    def s_wvT():
        wkvT_s[PR // 2:(PR + D) // 2, :] = _pk(wv_s[...].T)

    def xt(c):
        return x_s[pl.ds(c['r0'], T), :]

    def proj(lo, hi, c):
        return lax.dot_general(_upk(wkvT_s[lo // 2:hi // 2, :]), xt(c), NT_DIMS, preferred_element_type=f32)

    def s_pk(c):
        p = proj(0, PR, c)
        c['pka'], c['pkb'] = p[:PR // 2], p[PR // 2:]

    def s_pka(c):
        c['pka'] = proj(0, PR // 2, c)

    def s_pkb(c):
        c['pkb'] = proj(PR // 2, PR, c)

    def s_vt(c):
        c['vt'] = proj(PR, PR + D, c)

    def s_pv(c):
        p = proj(0, PR + D, c)
        c['pka'], c['pkb'], c['vt'] = p[:PR // 2], p[PR // 2:PR], p[PR:]

    def s_ln(c):
        c['ln'] = _ln_h(xt(c).astype(f32)).astype(bf16)

    def s_w1(c, c0=0, c1=NC):
        if 'ln' not in c:
            s_ln(c)
        hh = _gelu_h(jnp.dot(c['ln'], w1_s[:, c0 * 128:c1 * 128], preferred_element_type=f32))
        for k in range(c0, c1):
            h_s[k, pl.ds(c['r0'] + PAD, T), :] = hh[:, (k - c0) * 128:(k - c0 + 1) * 128]

    z_seen, kv_seen = set(), set()

    def sm_group(c, j):
        ep, en, sp, sn = _dual_exp(_group(c['pka'] if j < 4 else c['pkb'], j % 4))
        r = 1.0 / (sp * sn)
        php = ep * (r * sn)[None]
        phn = en * (r * sp)[None]
        ph = jnp.concatenate([php.reshape(64, T), phn.reshape(64, T)], axis=0)
        zz = ph[:, 0:128] + ph[:, 128:256]
        if j in z_seen:
            z_s[j] += zz
        else:
            z_s[j] = zz
            z_seen.add(j)
        c.setdefault('ph', {})[j] = ph.astype(bf16)

    def s_kv(c):
        for j in range(NG):
            if j not in c.get('ph', {}):
                sm_group(c, j)
            kk = lax.dot_general(c['vt'][j * 64:(j + 1) * 64].astype(bf16), c['ph'][j], NT_DIMS,
                                 preferred_element_type=f32)
            if j in kv_seen:
                kv_s[j] += kk
            else:
                kv_s[j] = kk
                kv_seen.add(j)

    def s_fin():
        kmask = (_iota((64, 128), 0) >> 4) == (_iota((64, 128), 1) & 3)
        for j in range(NG):
            kvT_s[j] = _pk(jnp.where(kmask, kv_s[j], 0.0).astype(bf16))
            z_s[j] = jnp.broadcast_to(jnp.sum(z_s[j], axis=1, keepdims=True), (128, 128))

    global_stage = dict(
        P1=s_p1, P2=s_p2, wvT=s_wvT, FIN=s_fin,
        fa=lambda: fold(wk_s, wkvT_s, 0, 2), fb=lambda: fold(wk_s, wkvT_s, 2, 4),
        fq=lambda: fold(wq_s, wqT_s, 0, 4))
    tile_stage = dict(
        pk=s_pk, pka=s_pka, pkb=s_pkb, vt=s_vt, pv=s_pv, ln=s_ln, w1=s_w1, kv=s_kv,
        w1a=lambda c: s_w1(c, 0, 2), w1b=lambda c: s_w1(c, 2, 4),
        sma=lambda c: [sm_group(c, j) for j in range(4)],
        smb=lambda c: [sm_group(c, j) for j in range(4, 8)])
    tiles = [dict(r0=k * T) for k in range(NT)]
    pending = iter(groups)
    for tok in PHASE1:
        if tok.startswith('W:'):
            for cp in next(pending):
                cp.wait()
        elif '.' in tok:
            name, k = tok.split('.')
            tile_stage[name](tiles[int(k)])
        else:
            global_stage[tok]()

    shifts = (-1, 1, -2, 2)

    def st_w2(c):
        r0 = c['r0']
        hsh = jnp.concatenate(
            [h_s[k, pl.ds(r0 + PAD + shifts[k], T), :] for k in range(NC)], axis=1).astype(bf16)
        c['x1'] = c['xt'].astype(f32) + jnp.dot(hsh, w2_s[...], preferred_element_type=f32)
        c['ln'] = _ln_h(c['x1']).astype(bf16)

    def st_w3m(c):
        u = lax.dot_general(c['ln'], w3_s[0:FM, :], NT_DIMS, preferred_element_type=f32)
        c['um'] = _gelu_h(u).astype(bf16)

    def st_w3t(c):
        ut = lax.dot_general(w3_s[FM:F, :], c['ln'], NT_DIMS, preferred_element_type=f32)
        ut = jnp.concatenate([_gelu_h(ut), jnp.zeros((128 - (F - FM), T), f32)], axis=0)
        c['ut'] = ut.T[:, :F - FM].astype(bf16)

    def st_pq(c):
        c['pqT'] = lax.dot_general(_upk(wqT_s[...]), c['xt'], NT_DIMS, preferred_element_type=f32)

    def st_oT(c):
        oTs = []
        for j in range(NG):
            ep, en, sp, sn = _dual_exp(_group(c['pqT'], j))
            z = jnp.concatenate([z_s[j]] * (T // 128), axis=1)
            zp = z[:64].reshape(8, 8, T)
            zn = z[64:].reshape(8, 8, T)
            dd = _fsum(ep * zp) * sn + (_fsum(en * zn) + 1e-6 * sn) * sp
            rd = 1.0 / dd
            php = ep * (sn * rd)[None]
            phn = en * (sp * rd)[None]
            ph = jnp.concatenate([php.reshape(64, T), phn.reshape(64, T)], axis=0).astype(bf16)
            oTs.append(jnp.dot(_upk(kvT_s[j]), ph, preferred_element_type=f32))
        hw = gate_s[...].astype(f32).reshape(1, D) * 0.5
        th = jnp.tanh(jnp.sum(c['xt'].astype(f32) * hw, axis=-1, keepdims=True))
        c['ng'] = 0.5 - 0.5 * th
        c['o'] = (jnp.concatenate(oTs, axis=0).T * (0.5 + 0.5 * th)).astype(bf16)

    def st_w4(c, key, nlo, nhi):
        u = jnp.concatenate([c['um'], c['ut']], axis=1)
        c[key] = c['x1'][:, nlo:nhi] + jnp.dot(u, w4_s[:, nlo:nhi], preferred_element_type=f32)

    def st_wo(c):
        b = jnp.concatenate([c['ba'], c['bb']], axis=1)
        cuts = CUTS if c['last'] else (0, T)
        for lo, hi in zip(cuts, cuts[1:]):
            a = jnp.dot(c['o'][lo:hi], wo_s[...], preferred_element_type=f32)
            rows = pl.ds(c['r0'] + lo, hi - lo)
            out_s[rows, :] = (b[lo:hi] * c['ng'][lo:hi] + a).astype(bf16)
            pltpu.make_async_copy(out_s.at[rows, :], out_hbm.at[0, rows, :], sems.at[0]).start()

    stage2 = dict(w2=st_w2, w3m=st_w3m, w3t=st_w3t, pq=st_pq, oT=st_oT, wo=st_wo,
                  w4a=lambda c: st_w4(c, 'ba', 0, HD), w4b=lambda c: st_w4(c, 'bb', HD, D))

    def phase2(i, carry):
        cs = []
        for k in range(TILES_PER_STEP):
            r0 = pl.multiple_of((i * TILES_PER_STEP + k) * T, T)
            cs.append(dict(r0=r0, xt=x_s[pl.ds(r0, T), :], last=(k == TILES_PER_STEP - 1)))
        for tok in PHASE2:
            name, k = tok.split('.')
            stage2[name](cs[int(k)])
        return carry

    lax.fori_loop(0, NT // TILES_PER_STEP, phase2, 0)
    pltpu.make_async_copy(out_s, out_hbm.at[0], sems.at[0]).wait()


@jax.jit
def pallas_gated_mix__linear_kernel_hedgehog__mixer_s_mlp__prompt_kernel(
    A_x: jax.Array,
    A_wqkv: jax.Array,
    A_w_phi: jax.Array,
    A_wo: jax.Array,
    B_x: jax.Array,
    B_w1: jax.Array,
    B_w2: jax.Array,
    B_w3: jax.Array,
    B_w4: jax.Array,
    gate_w: jax.Array,
):
    del B_x
    hbm = pl.BlockSpec(memory_space=pltpu.HBM)
    return pl.pallas_call(
        _kernel,
        out_shape=jax.ShapeDtypeStruct((1, S, D), bf16),
        in_specs=[hbm] * 9,
        out_specs=hbm,
        scratch_shapes=[
            pltpu.VMEM((S, D), bf16),
            pltpu.VMEM((D, D), bf16), pltpu.VMEM((D, D), bf16), pltpu.VMEM((D, D), bf16),
            pltpu.VMEM((DH, DH, H), bf16),
            pltpu.VMEM((D, D), bf16), pltpu.VMEM((D, D), bf16), pltpu.VMEM((D, D), bf16),
            pltpu.VMEM((F, D), bf16), pltpu.VMEM((F, D), bf16),
            pltpu.VMEM((D,), bf16),
            pltpu.VMEM((PR // 2, D), u32), pltpu.VMEM(((PR + D) // 2, D), u32),
            pltpu.VMEM((NC, S + 2 * PAD, 128), f32),
            pltpu.VMEM((NG, 64, 128), f32),
            pltpu.VMEM((NG, 128, 128), f32),
            pltpu.VMEM((NG, 32, 128), u32),
            pltpu.VMEM((S, D), bf16),
            pltpu.VMEM((NC, 128, 128), bf16),
            pltpu.SemaphoreType.DMA((NSEM,)),
        ],
        compiler_params=pltpu.CompilerParams(
            vmem_limit_bytes=64 * 1024 * 1024,
            disable_bounds_checks=True,
            disable_semaphore_checks=True,
        ),
    )(A_x, A_wqkv, jnp.transpose(A_w_phi, (1, 2, 0)), A_wo, B_w1, B_w2, B_w3.T, B_w4, gate_w)
```

```python
import jax
import jax.numpy as jnp
from jax import lax
import jax.experimental.pallas as pl
import jax.experimental.pallas.tpu as pltpu

S, D, H, DH, F = 2048, 512, 32, 16, 1376
NC = D // 128
NG = 8
T = 256
NT = S // T
CUTS = (0, 128, 192, 224, 256)
PAD = 8
PR = 480
FM = 1280
HD = D // 2
LOG2E = 1.4426950408889634
GC1 = 0.7978845608028654
GC2 = GC1 * 0.044715
NT_DIMS = (((1,), (1,)), ((), ()))
f32, bf16 = jnp.float32, jnp.bfloat16

PHASE1 = (
    'W:wphi,P1,W:x0-1,P2,ln.0,W:w1a,w1a.0,W:wka,fa,pka.0,sma.0,W:wkb+w1b,fb,pkb.0,w1b.0,smb.0,'
    'W:x1-2+wv,wvT,pk.1,vt.1,vt.0,w1a.1,kv.0,kv.1,W:x2-8+wq,w1b.1,vt.2,w1a.2,pk.2,w1b.2,pv.3,w1.3,kv.2,'
    'w1a.4,w1b.4,kv.3,pv.4,pv.5,w1a.5,w1b.5,kv.4,pv.6,w1b.6,fq,w1a.6,kv.5,kv.6,w1.7,pv.7,kv.7,'
    'FIN,W:w2+w3+w4+wo+gate').split(',')
PHASE2 = (
    'w2.0,w2.1,w3m.0,pq.0,w3t.0,w4b.0,w4a.0,oT.0,w2.2,w3t.1,wo.0,w3m.1,w4a.1,pq.1,w4b.1,oT.1,'
    'w2.3,w3m.2,w3t.2,wo.1,w4a.2,pq.2,w4b.2,oT.2,w3t.3,w3m.3,pq.3,wo.2,w4a.3,oT.3,w4b.3,wo.3').split(',')
TILES_PER_STEP = 4
NSEM = sum(t.startswith('W:') for t in PHASE1)


def _iota(shape, dim):
    return lax.broadcasted_iota(jnp.int32, shape, dim)


def _gelu_h(v):
    return v + v * jnp.tanh(v * (2.0 * GC1 + (8.0 * GC2) * (v * v)))


def _ln_h(u):
    m = jnp.sum(u, axis=-1, keepdims=True) * (1.0 / D)
    v = jnp.maximum(jnp.sum(u * u, axis=-1, keepdims=True) * (1.0 / D) - m * m, 0.0) + 1e-5
    return (u - m) * jnp.exp2(jnp.log2(v) * -0.5 - 1.0)


def _fsum(e):
    s = jnp.sum(e, axis=0)
    return s + pltpu.roll(s, 4, 0)


def _group(p, j):
    n = p.shape[-1]
    c, g2 = j // 2, j % 2
    main = p[c * 120 + g2 * 64:c * 120 + g2 * 64 + 56].reshape(7, 8, n)
    sub = _iota((8, n), 0)
    keep = (sub < 4) if g2 == 0 else (sub >= 4)
    last = jnp.where(keep, p[c * 120 + 56:c * 120 + 64], 0.0)
    return jnp.concatenate([main, last[None]], axis=0)


def _dual_exp(p3):
    mx = jnp.max(p3, axis=0)
    mx = jnp.maximum(mx, pltpu.roll(mx, 4, 0))
    mn = jnp.min(p3, axis=0)
    mn = jnp.minimum(mn, pltpu.roll(mn, 4, 0))
    ep = jnp.exp2(p3 - mx[None])
    en = jnp.exp2(mn[None] - p3)
    return ep, en, _fsum(ep), _fsum(en)


def _kernel(x_hbm, wqkv_hbm, wphi_hbm, wo_hbm, w1_hbm, w2_hbm, w3_hbm, w4_hbm, gate_hbm,
            out_hbm,
            x_s, wq_s, wk_s, wv_s, wphi_s, wo_s, w1_s, w2_s, w3_s, w4_s, gate_s,
            wqT_s, wkvT_s, h_s, kv_s, z_s, kvT_s, out_s, pt_s,
            sems):
    def in_copy(name, sem):
        if name[0] == 'x':
            a, b = (int(v) for v in name[1:].split('-'))
            rows = pl.ds(a * T, (b - a) * T)
            return pltpu.make_async_copy(x_hbm.at[0, rows, :], x_s.at[rows, :], sem)
        src, dst = dict(
            wphi=(wphi_hbm, wphi_s),
            wka=(wqkv_hbm.at[:, pl.ds(D, HD)], wk_s.at[:, pl.ds(0, HD)]),
            wkb=(wqkv_hbm.at[:, pl.ds(D + HD, HD)], wk_s.at[:, pl.ds(HD, HD)]),
            wv=(wqkv_hbm.at[:, pl.ds(2 * D, D)], wv_s),
            wq=(wqkv_hbm.at[:, pl.ds(0, D)], wq_s),
            w1a=(w1_hbm.at[:, pl.ds(0, HD)], w1_s.at[:, pl.ds(0, HD)]),
            w1b=(w1_hbm.at[:, pl.ds(HD, HD)], w1_s.at[:, pl.ds(HD, HD)]),
            w2=(w2_hbm, w2_s), w3=(w3_hbm, w3_s), w4=(w4_hbm, w4_s), wo=(wo_hbm, wo_s),
            gate=(gate_hbm, gate_s),
        )[name]
        return pltpu.make_async_copy(src, dst, sem)

    waits = [t for t in PHASE1 if t.startswith('W:')]
    groups = [[in_copy(n, sems.at[i]) for n in t[2:].split('+')] for i, t in enumerate(waits)]
    for grp in groups:
        for cp in grp:
            cp.start()

    h_s[:, pl.ds(0, PAD), :] = jnp.zeros((NC, PAD, 128), f32)
    h_s[:, pl.ds(PAD + S, PAD), :] = jnp.zeros((NC, PAD, 128), f32)

    tmp = {}

    def s_p1():
        sel = jnp.where(_iota((H, D), 0) == (_iota((H, D), 1) >> 4), 1.0, 0.0).astype(bf16)
        dmask = (_iota((256, D), 0) >> 4) == (_iota((256, D), 1) & 15)
        a2d = wphi_s[...].reshape(DH * DH, H)
        tmp['bm'] = jnp.where(dmask, jnp.dot(a2d, sel, preferred_element_type=f32), 0.0).astype(bf16)

    def s_p2():
        row = _iota((128, 128), 0)
        head_mask = ((row >> 6) * 4 + (row & 3)) == (_iota((128, 128), 1) >> 4)
        e2 = jnp.where(((_iota((128, 256), 0) & 63) >> 2) == (_iota((128, 256), 1) & 15), 1.0, 0.0).astype(bf16)
        pall = jnp.dot(e2, tmp['bm'], preferred_element_type=f32)
        for c in range(NC):
            pt_s[c] = jnp.where(head_mask, pall[:, c * 128:(c + 1) * 128], 0.0).astype(bf16)

    def fold(w_s, wT_s, c0, c1):
        lo = _iota((8, D), 0) < 4
        rows = []
        for c in range(c0, c1):
            r = lax.dot_general(pt_s[c], w_s[:, c * 128:(c + 1) * 128], NT_DIMS,
                                preferred_element_type=f32) * LOG2E
            a7, b7 = r[56:64], r[120:128]
            a7r, b7r = pltpu.roll(a7, 4, 0), pltpu.roll(b7, 4, 0)
            ra = jnp.where(lo, a7r, a7)
            rb = jnp.where(lo, b7, b7r)
            rows.append((r[0:56].reshape(7, 8, D) - ra[None]).reshape(56, D))
            rows.append(jnp.where(lo, a7 - a7r, b7 - b7r))
            rows.append((r[64:120].reshape(7, 8, D) - rb[None]).reshape(56, D))
        wT_s[c0 * 120:c1 * 120, :] = jnp.concatenate(rows, axis=0).astype(bf16)

    def s_wvT():
        wkvT_s[PR:PR + D, :] = wv_s[...].T

    def xt(c):
        return x_s[pl.ds(c['r0'], T), :]

    def proj(lo, hi, c):
        return lax.dot_general(wkvT_s[lo:hi, :], xt(c), NT_DIMS, preferred_element_type=f32)

    def s_pk(c):
        p = proj(0, PR, c)
        c['pka'], c['pkb'] = p[:PR // 2], p[PR // 2:]

    def s_pka(c):
        c['pka'] = proj(0, PR // 2, c)

    def s_pkb(c):
        c['pkb'] = proj(PR // 2, PR, c)

    def s_vt(c):
        c['vt'] = proj(PR, PR + D, c)

    def s_pv(c):
        p = proj(0, PR + D, c)
        c['pka'], c['pkb'], c['vt'] = p[:PR // 2], p[PR // 2:PR], p[PR:]

    def s_ln(c):
        c['ln'] = _ln_h(xt(c).astype(f32)).astype(bf16)

    def s_w1(c, c0=0, c1=NC):
        if 'ln' not in c:
            s_ln(c)
        hh = _gelu_h(jnp.dot(c['ln'], w1_s[:, c0 * 128:c1 * 128], preferred_element_type=f32))
        for k in range(c0, c1):
            h_s[k, pl.ds(c['r0'] + PAD, T), :] = hh[:, (k - c0) * 128:(k - c0 + 1) * 128]

    z_seen, kv_seen = set(), set()

    def sm_group(c, j):
        ep, en, sp, sn = _dual_exp(_group(c['pka'] if j < 4 else c['pkb'], j % 4))
        r = 1.0 / (sp * sn)
        php = ep * (r * sn)[None]
        phn = en * (r * sp)[None]
        ph = jnp.concatenate([php.reshape(64, T), phn.reshape(64, T)], axis=0)
        zz = ph[:, 0:128] + ph[:, 128:256]
        if j in z_seen:
            z_s[j] += zz
        else:
            z_s[j] = zz
            z_seen.add(j)
        c.setdefault('ph', {})[j] = ph.astype(bf16)

    def s_kv(c):
        for j in range(NG):
            if j not in c.get('ph', {}):
                sm_group(c, j)
            kk = lax.dot_general(c['vt'][j * 64:(j + 1) * 64].astype(bf16), c['ph'][j], NT_DIMS,
                                 preferred_element_type=f32)
            if j in kv_seen:
                kv_s[j] += kk
            else:
                kv_s[j] = kk
                kv_seen.add(j)

    def s_fin():
        kmask = (_iota((64, 128), 0) >> 4) == (_iota((64, 128), 1) & 3)
        for j in range(NG):
            kvT_s[j] = jnp.where(kmask, kv_s[j], 0.0).astype(bf16)
            z_s[j] = jnp.broadcast_to(jnp.sum(z_s[j], axis=1, keepdims=True), (128, 128))

    global_stage = dict(
        P1=s_p1, P2=s_p2, wvT=s_wvT, FIN=s_fin,
        fa=lambda: fold(wk_s, wkvT_s, 0, 2), fb=lambda: fold(wk_s, wkvT_s, 2, 4),
        fq=lambda: fold(wq_s, wqT_s, 0, 4))
    tile_stage = dict(
        pk=s_pk, pka=s_pka, pkb=s_pkb, vt=s_vt, pv=s_pv, ln=s_ln, w1=s_w1, kv=s_kv,
        w1a=lambda c: s_w1(c, 0, 2), w1b=lambda c: s_w1(c, 2, 4),
        sma=lambda c: [sm_group(c, j) for j in range(4)],
        smb=lambda c: [sm_group(c, j) for j in range(4, 8)])
    tiles = [dict(r0=k * T) for k in range(NT)]
    pending = iter(groups)
    for tok in PHASE1:
        if tok.startswith('W:'):
            for cp in next(pending):
                cp.wait()
        elif '.' in tok:
            name, k = tok.split('.')
            tile_stage[name](tiles[int(k)])
        else:
            global_stage[tok]()

    shifts = (-1, 1, -2, 2)

    def st_w2(c):
        r0 = c['r0']
        hsh = jnp.concatenate(
            [h_s[k, pl.ds(r0 + PAD + shifts[k], T), :] for k in range(NC)], axis=1).astype(bf16)
        c['x1'] = c['xt'].astype(f32) + jnp.dot(hsh, w2_s[...], preferred_element_type=f32)
        c['ln'] = _ln_h(c['x1']).astype(bf16)

    def st_w3m(c):
        u = lax.dot_general(c['ln'], w3_s[0:FM, :], NT_DIMS, preferred_element_type=f32)
        c['um'] = _gelu_h(u).astype(bf16)

    def st_w3t(c):
        ut = lax.dot_general(w3_s[FM:F, :], c['ln'], NT_DIMS, preferred_element_type=f32)
        ut = jnp.concatenate([_gelu_h(ut), jnp.zeros((128 - (F - FM), T), f32)], axis=0)
        c['ut'] = ut.T[:, :F - FM].astype(bf16)

    def st_pq(c):
        c['pqT'] = lax.dot_general(wqT_s[...], c['xt'], NT_DIMS, preferred_element_type=f32)

    def st_oT(c):
        oTs = []
        for j in range(NG):
            ep, en, sp, sn = _dual_exp(_group(c['pqT'], j))
            z = jnp.concatenate([z_s[j]] * (T // 128), axis=1)
            zp = z[:64].reshape(8, 8, T)
            zn = z[64:].reshape(8, 8, T)
            dd = _fsum(ep * zp) * sn + (_fsum(en * zn) + 1e-6 * sn) * sp
            rd = 1.0 / dd
            php = ep * (sn * rd)[None]
            phn = en * (sp * rd)[None]
            ph = jnp.concatenate([php.reshape(64, T), phn.reshape(64, T)], axis=0).astype(bf16)
            oTs.append(jnp.dot(kvT_s[j], ph, preferred_element_type=f32))
        hw = gate_s[...].astype(f32).reshape(1, D) * 0.5
        th = jnp.tanh(jnp.sum(c['xt'].astype(f32) * hw, axis=-1, keepdims=True))
        c['ng'] = 0.5 - 0.5 * th
        c['o'] = (jnp.concatenate(oTs, axis=0).T * (0.5 + 0.5 * th)).astype(bf16)

    def st_w4(c, key, nlo, nhi):
        u = jnp.concatenate([c['um'], c['ut']], axis=1)
        c[key] = c['x1'][:, nlo:nhi] + jnp.dot(u, w4_s[:, nlo:nhi], preferred_element_type=f32)

    def st_wo(c):
        b = jnp.concatenate([c['ba'], c['bb']], axis=1)
        cuts = CUTS if c['last'] else (0, T)
        for lo, hi in zip(cuts, cuts[1:]):
            a = jnp.dot(c['o'][lo:hi], wo_s[...], preferred_element_type=f32)
            rows = pl.ds(c['r0'] + lo, hi - lo)
            out_s[rows, :] = (b[lo:hi] * c['ng'][lo:hi] + a).astype(bf16)
            pltpu.make_async_copy(out_s.at[rows, :], out_hbm.at[0, rows, :], sems.at[0]).start()

    stage2 = dict(w2=st_w2, w3m=st_w3m, w3t=st_w3t, pq=st_pq, oT=st_oT, wo=st_wo,
                  w4a=lambda c: st_w4(c, 'ba', 0, HD), w4b=lambda c: st_w4(c, 'bb', HD, D))

    def phase2(i, carry):
        cs = []
        for k in range(TILES_PER_STEP):
            r0 = pl.multiple_of((i * TILES_PER_STEP + k) * T, T)
            cs.append(dict(r0=r0, xt=x_s[pl.ds(r0, T), :], last=(k == TILES_PER_STEP - 1)))
        for tok in PHASE2:
            name, k = tok.split('.')
            stage2[name](cs[int(k)])
        return carry

    lax.fori_loop(0, NT // TILES_PER_STEP, phase2, 0)
    pltpu.make_async_copy(out_s, out_hbm.at[0], sems.at[0]).wait()


@jax.jit
def pallas_gated_mix__linear_kernel_hedgehog__mixer_s_mlp__prompt_kernel(
    A_x: jax.Array,
    A_wqkv: jax.Array,
    A_w_phi: jax.Array,
    A_wo: jax.Array,
    B_x: jax.Array,
    B_w1: jax.Array,
    B_w2: jax.Array,
    B_w3: jax.Array,
    B_w4: jax.Array,
    gate_w: jax.Array,
):
    del B_x
    hbm = pl.BlockSpec(memory_space=pltpu.HBM)
    return pl.pallas_call(
        _kernel,
        out_shape=jax.ShapeDtypeStruct((1, S, D), bf16),
        in_specs=[hbm] * 9,
        out_specs=hbm,
        scratch_shapes=[
            pltpu.VMEM((S, D), bf16),
            pltpu.VMEM((D, D), bf16), pltpu.VMEM((D, D), bf16), pltpu.VMEM((D, D), bf16),
            pltpu.VMEM((DH, DH, H), bf16),
            pltpu.VMEM((D, D), bf16), pltpu.VMEM((D, D), bf16), pltpu.VMEM((D, D), bf16),
            pltpu.VMEM((F, D), bf16), pltpu.VMEM((F, D), bf16),
            pltpu.VMEM((D,), bf16),
            pltpu.VMEM((PR, D), bf16), pltpu.VMEM((PR + D, D), bf16),
            pltpu.VMEM((NC, S + 2 * PAD, 128), f32),
            pltpu.VMEM((NG, 64, 128), f32),
            pltpu.VMEM((NG, 128, 128), f32),
            pltpu.VMEM((NG, 64, 128), bf16),
            pltpu.VMEM((S, D), bf16),
            pltpu.VMEM((NC, 128, 128), bf16),
            pltpu.SemaphoreType.DMA((NSEM,)),
        ],
        compiler_params=pltpu.CompilerParams(
            vmem_limit_bytes=64 * 1024 * 1024,
            disable_bounds_checks=True,
            disable_semaphore_checks=True,
        ),
    )(A_x, A_wqkv, jnp.transpose(A_w_phi, (1, 2, 0)), A_wo, B_w1, B_w2, B_w3.T, B_w4, gate_w)
```
